```python
import jax
import jax.numpy as jnp

def _softmax(x, axis=-1):
    return jax.nn.softmax(x, axis=axis)
def _gelu(x):
    return jax.nn.gelu(x, approximate=True)
def _silu(x):
    return jax.nn.silu(x)
def _sigmoid(x):
    return jax.nn.sigmoid(x)
def _layernorm(x, axis=-1, eps=1e-5):
    m = jnp.mean(x, axis=axis, keepdims=True)
    v = jnp.var(x, axis=axis, keepdims=True)
    return (x - m) / jnp.sqrt(v + eps)
def _scatter_add(tgt, idx, src, axis=0):
    return tgt.at[idx].add(src)
def _segment_sum(src, seg, n):
    return jax.ops.segment_sum(src, seg, n)
class _Rng:
    def __init__(self, key):
        self._k = key
    def _next(self):
        self._k, sub = jax.random.split(self._k)
        return sub
    def normal(self, shape):
        return jax.random.normal(self._next(), shape, dtype=jnp.bfloat16)
    def randint(self, lo, hi, shape):
        return jax.random.randint(self._next(), shape, lo, hi, dtype=jnp.int32)
    def uniform(self, shape, lo=0.0, hi=1.0):
        return jax.random.uniform(self._next(), shape, jnp.bfloat16, lo, hi)
    def permutation(self, n):
        return jax.random.permutation(self._next(), n)


kernel_name = 'recurrent_scan__sliding_block_cached__dense_activation_gelu__decode'

def setup_inputs():
    _rng = _Rng(jax.random.key(int.from_bytes(__import__("os").urandom(4), "little")))
    _w = (lambda a: (lambda t: t.astype(jnp.bfloat16) if jnp.issubdtype(t.dtype, jnp.floating) else t)(jnp.asarray(a)))
    def _A_setup():
        B, Sq, D = 2, 1, 576
        Hq, Hkv, Sk, Dh = 32, 16, 32768, 128
        assert Hq % Hkv == 0, (Hq, Hkv)
        return {
            "x": _w((lambda *s: _rng.normal(s) * 0.05)(B, Sq, D)),
            "k_cache": _w((lambda *s: _rng.normal(s) * 0.05)(B, Hkv, Sk, Dh)),
            "v_cache": _w((lambda *s: _rng.normal(s) * 0.05)(B, Hkv, Sk, Dh)),
            "wq": _w((lambda *s: _rng.normal(s) * 0.05)(D, Hq * Dh) * (D ** -0.5)),
            "wo": _w((lambda *s: _rng.normal(s) * 0.05)(Hq * Dh, D) * ((Hq * Dh) ** -0.5)),
        }
    _A_in = _A_setup()

    def _B_setup():
        B, S, D, F = 2, 1, 576, 4608
        return {
            "x": _w((lambda *s: _rng.normal(s) * 0.05)(B, S, D)),
            "w1": _w((lambda *s: _rng.normal(s) * 0.05)(D, F) * (D ** -0.5)),
            "b1": _w((lambda *s: _rng.normal(s) * 0.05)(F) * 0.01),
            "w2": _w((lambda *s: _rng.normal(s) * 0.05)(F, D) * (F ** -0.5)),
            "b2": _w((lambda *s: _rng.normal(s) * 0.05)(D) * 0.01),
        }
    _B_in = _B_setup()

    return {
        "A_x": _A_in["x"],
        "A_k_cache": _A_in["k_cache"],
        "A_v_cache": _A_in["v_cache"],
        "A_wq": _A_in["wq"],
        "A_wo": _A_in["wo"],
        "B_x": _B_in["x"],
        "B_w1": _B_in["w1"],
        "B_b1": _B_in["b1"],
        "B_w2": _B_in["w2"],
        "B_b2": _B_in["b2"],
    }

def reference(A_x, A_k_cache, A_v_cache, A_wq, A_wo, B_x, B_w1, B_b1, B_w2, B_b2):
    def _A_ref(x, k_cache, v_cache, wq, wo):
        B, Sq, D = x.shape
        Hq, Dh = 32, 128
        Hkv, Sk = k_cache.shape[1], k_cache.shape[2]
        W = min(4096, max(256, Sk // 4))
        rep = Hq // Hkv
        q = (lambda x, *d: x.transpose(*d))((x @ wq).reshape(B, Sq, Hq, Dh), 0, 2, 1, 3)
        k = jnp.repeat(k_cache[:, :, Sk - W:, :], rep, axis=1)
        v = jnp.repeat(v_cache[:, :, Sk - W:, :], rep, axis=1)
        scores = jnp.einsum("bhqd,bhkd->bhqk", q, k) * (Dh ** -0.5)
        p = _softmax(scores, axis=-1)
        o = jnp.einsum("bhqk,bhkd->bhqd", p, v)
        return (lambda x, *d: x.transpose(*d))(o, 0, 2, 1, 3).reshape(B, Sq, Hq * Dh) @ wo

    def _B_ref(x, w1, b1, w2, b2):
        h = jnp.einsum("bsd,df->bsf", x, w1) + b1
        h = _gelu(h)
        return jnp.einsum("bsf,fd->bsd", h, w2) + b2

    x = A_x
    xn = _layernorm(x, axis=-1)
    s = _A_ref(xn, A_k_cache, A_v_cache, A_wq, A_wo)
    g = _silu(_B_ref(xn, B_w1, B_b1, B_w2, B_b2))
    return x + s * g
```

```python
import functools
import jax
import jax.numpy as jnp
from jax import lax
from jax.experimental import pallas as pl
from jax.experimental.pallas import tpu as pltpu

B, D, HQ, HKV, SK, DH, F = 2, 576, 32, 16, 32768, 128, 4608
W = 4096
NT = (((1,), (1,)), ((), ()))
NN = (((1,), (0,)), ((), ()))
bf = jnp.bfloat16
f32 = jnp.float32

NJ = 4
CR = 256
UR = NJ * CR
WR = 8
T_WQ, T_W1, T_WO, T_KV, T_W2, T_END = 0, 9, 18, 27, 155, 164


def make(no_dma=False, no_compute=False, A0=1, A1=4, checks=True):
    R0, R1 = A0 + 1, A1 + 1
    AH = (A0, A1)

    def kernel(x_hbm, k_hbm, v_hbm, wq_hbm, woT_hbm, w1_hbm, b1_hbm, w2T_hbm, b2_hbm, o_hbm,
               kbuf, vbuf, wqb, wob, w1b, w2b, xb, b1b, b2b, ob,
               x8b, qs, sc, pb, lsum, acc, sacc, hb, yb, b1f,
               sem0, sem1, semx):
        sems = (sem0, sem1)
        RR = (R0, R1)

        def wcopy(src, dst, s, i, j, t):
            r0 = pl.multiple_of(64 * i + 32 * s + WR * j, WR)
            return pltpu.make_async_copy(src.at[pl.ds(r0, WR), :], dst.at[pl.ds(r0, WR), :], sems[s].at[t % RR[s]])

        def kvcopy(s, n, j, t):
            h = n // 8
            b = (n // 4) % 2
            r0 = pl.multiple_of((n % 4) * UR + j * CR, CR)
            src, dst = ((k_hbm, kbuf), (v_hbm, vbuf))[s]
            return pltpu.make_async_copy(src.at[b, h, pl.ds(SK - W + r0, CR), :], dst.at[h, b, pl.ds(r0, CR), :],
                                         sems[s].at[t % RR[s]])

        segs = [
            (T_WQ, T_W1, lambda s, t, j: wcopy(wq_hbm, wqb, s, t - T_WQ, j, t)),
            (T_W1, T_WO, lambda s, t, j: wcopy(w1_hbm, w1b, s, t - T_W1, j, t)),
            (T_WO, T_KV, lambda s, t, j: wcopy(woT_hbm, wob, s, t - T_WO, j, t)),
            (T_KV, T_W2, lambda s, t, j: kvcopy(s, t - T_KV, j, t)),
            (T_W2, T_END, lambda s, t, j: wcopy(w2T_hbm, w2b, s, t - T_W2, j, t)),
        ]

        def for_seg(t, lo, hi, fn):
            for (b_, e_, mk) in segs:
                if e_ <= lo or b_ > hi:
                    continue
                if b_ <= lo and hi < e_:
                    fn(mk)
                elif isinstance(t, int):
                    if b_ <= t < e_:
                        fn(mk)
                else:
                    conds = []
                    if lo < b_:
                        conds.append(t >= b_)
                    if hi >= e_:
                        conds.append(t < e_)
                    c = conds[0] if len(conds) == 1 else jnp.logical_and(conds[0], conds[1])
                    pl.when(c)(functools.partial(fn, mk))

        def start(s, t, j, lo, hi):
            if no_dma:
                return
            for_seg(t, lo, hi, lambda mk: mk(s, t, j).start(priority=s))

        def wait(s, t, j, lo, hi):
            if no_dma:
                return
            for_seg(t, lo, hi, lambda mk: mk(s, t, j).wait())

        def pair(t, j, lo, hi):
            wait(1, t, j, lo, hi)
            start(0, t + A0, j, lo + A0, hi + A0)
            wait(0, t, j, lo, hi)
            start(1, t + A1, j, lo + A1, hi + A1)

        def unit(t, lo, hi, slot_a=None, slot_b=None):
            pair(t, 0, lo, hi)
            pair(t, 1, lo, hi)
            if slot_a is not None and not no_compute:
                slot_a()
            pair(t, 2, lo, hi)
            pair(t, 3, lo, hi)
            if slot_b is not None and not no_compute:
                slot_b()

        cx = pltpu.make_async_copy(x_hbm, xb, semx.at[0])
        cb1 = pltpu.make_async_copy(b1_hbm, b1b, semx.at[0])
        cb2 = pltpu.make_async_copy(b2_hbm, b2b, semx.at[0])
        if not no_dma:
            for t in range(A0):
                for j in range(NJ):
                    start(0, t, j, t, t)
            cx.start(); cb1.start(); cb2.start()
            for t in range(A1):
                for j in range(NJ):
                    start(1, t, j, t, t)
            cx.wait(); cb1.wait(); cb2.wait()

        row128 = lax.broadcasted_iota(jnp.int32, (8, DH), 0)

        x = xb[...].astype(f32)
        mu = jnp.mean(x, axis=-1, keepdims=True)
        xc = x - mu
        var = jnp.mean(xc * xc, axis=-1, keepdims=True)
        xn = xc / jnp.sqrt(var + 1e-5)
        rowd = lax.broadcasted_iota(jnp.int32, (8, D), 0)
        x8b[...] = jnp.where(rowd % 2 == 0, jnp.broadcast_to(xn[0:1], (8, D)), jnp.broadcast_to(xn[1:2], (8, D))).astype(bf)

        bias1 = b1b[...].astype(f32)
        for j in range(F // 128):
            b1f[:, pl.ds(128 * j, 128)] = jnp.broadcast_to(bias1[j:j + 1, :], (8, 128))

        def qproj(h):
            c0 = pl.multiple_of(h * 256, 256)
            q = lax.dot_general(x8b[...], wqb[:, pl.ds(c0, 256)], NN, preferred_element_type=f32)
            qs[h] = jnp.where(row128 < 2, q[:, :128], q[:, 128:]).astype(bf)

        def ffn1(p):
            c0 = pl.multiple_of(p * 256, 256)
            hh = lax.dot_general(x8b[...], w1b[:, pl.ds(c0, 256)], NN, preferred_element_type=f32)
            hh = hh + b1f[:, pl.ds(c0, 256)]
            hb[:, pl.ds(c0, 256)] = jax.nn.gelu(hh, approximate=True).astype(bf)

        def qk(h, k):
            b, u = k // 4, k % 4
            s = lax.dot_general(qs[h], kbuf[h, b, pl.ds(u * UR, UR), :], NT, preferred_element_type=f32)
            sc[b, :, pl.ds(u * UR, UR)] = s

        def softmax():
            roww = lax.broadcasted_iota(jnp.int32, (8, W), 0)
            s = jnp.where(roww % 2 == 0, sc[0], sc[1]) * (DH ** -0.5)
            m = jnp.max(s, axis=-1, keepdims=True)
            p = jnp.exp(s - m)
            l = jnp.sum(p, axis=-1, keepdims=True)
            lsum[...] = jnp.broadcast_to(l, (8, DH))
            pb[...] = p.astype(bf)

        def pv(h, k):
            b, u = k // 4, k % 4
            o = lax.dot_general(pb[:, pl.ds(u * UR, UR)], vbuf[h, b, pl.ds(u * UR, UR), :], NN, preferred_element_type=f32)
            if u == 0:
                acc[b] = o
            else:
                acc[b] = acc[b] + o

        def finalize(h):
            o = jnp.where(row128 % 2 == 0, acc[0], acc[1]) / lsum[...]
            la = jnp.where(row128 < 2, o, 0.0)
            lb = jnp.where((row128 >= 2) & (row128 < 4), o, 0.0)
            L = jnp.concatenate([la, lb], axis=1).astype(bf)
            c0 = pl.multiple_of(h * 256, 256)
            sacc[...] += lax.dot_general(L, wob[:, pl.ds(c0, 256)], NT, preferred_element_type=f32)

        def ffn2(p):
            n = 128 if p < 4 else 64
            y = lax.dot_general(hb[...], w2b[pl.ds(128 * p, n), :], NT, preferred_element_type=f32)
            yb[:, pl.ds(128 * p, n)] = y

        sacc[...] = jnp.zeros(sacc.shape, f32)

        def body1a(t, c):
            unit(t, T_WQ, T_W1 - 1)
            return c
        lax.fori_loop(T_WQ, T_W1, body1a, 0)

        def body1b(t, c):
            i = t - T_W1
            def sa():
                pl.when(i < 8)(lambda: qproj(2 * i))
            def sb():
                pl.when(i < 8)(lambda: qproj(2 * i + 1))
            unit(t, T_W1, T_WO - 1, sa, sb)
            return c
        lax.fori_loop(T_W1, T_WO, body1b, 0)

        def body1c(t, c):
            i = t - T_WO
            unit(t, T_WO, T_KV - 1, lambda: ffn1(2 * i), lambda: ffn1(2 * i + 1))
            return c
        lax.fori_loop(T_WO, T_KV, body1c, 0)

        def body2(h, c):
            for k in range(8):
                t = T_KV + 8 * h + k
                lo, hi = T_KV + k, T_KV + 8 * 15 + k
                if k == 0:
                    def sa():
                        @pl.when(h > 0)
                        def _():
                            qk(h - 1, 7)
                            softmax()
                else:
                    sa = functools.partial(qk, h, k - 1)

                def sb(k=k):
                    @pl.when(h > 0)
                    def _():
                        pv(h - 1, k)
                        if k == 7:
                            finalize(h - 1)
                unit(t, lo, hi, sa, sb)
            return c
        lax.fori_loop(0, HKV, body2, 0)

        h = HKV - 1
        def a0():
            qk(h, 7); softmax()
        def b0():
            for k in range(4): pv(h, k)
        def a1():
            for k in range(4, 8): pv(h, k)
        def b1_():
            finalize(h)
        slots = {0: (a0, b0), 1: (a1, b1_), 2: (lambda: ffn2(0), None), 4: (lambda: ffn2(1), None),
                 6: (lambda: ffn2(2), None), 8: (lambda: ffn2(3), None)}
        for i in range(T_END - T_W2):
            t = T_W2 + i
            sa, sb = slots.get(i, (None, None))
            unit(t, t, t, sa, sb)
        if not no_compute:
            ffn2(4)
            y = yb[0:2, :] + b2b[...].astype(f32).reshape(1, D)
            g = y * jax.nn.sigmoid(y)
            s8 = sacc[...]
            sres = s8[0:2] + s8[2:4]
            ob[...] = (x + sres * g).astype(bf)
        else:
            ob[...] = x.astype(bf)
        oc = pltpu.make_async_copy(ob, o_hbm, semx.at[0])
        oc.start(); oc.wait()

    @jax.jit
    def fn(A_x, A_k_cache, A_v_cache, A_wq, A_wo, B_x, B_w1, B_b1, B_w2, B_b2):
        hbm = pl.BlockSpec(memory_space=pltpu.HBM)
        out = pl.pallas_call(
            kernel,
            out_shape=jax.ShapeDtypeStruct((B, D), bf),
            in_specs=[hbm] * 9,
            out_specs=hbm,
            scratch_shapes=[
                pltpu.VMEM((HKV, B, W, DH), bf), pltpu.VMEM((HKV, B, W, DH), bf),
                pltpu.VMEM((D, HQ * DH), bf), pltpu.VMEM((D, HQ * DH), bf),
                pltpu.VMEM((D, F), bf), pltpu.VMEM((D, F), bf),
                pltpu.VMEM((B, D), bf), pltpu.VMEM((F // 128, 128), bf), pltpu.VMEM((D,), bf),
                pltpu.VMEM((B, D), bf),
                pltpu.VMEM((8, D), bf),
                pltpu.VMEM((HKV, 8, DH), bf),
                pltpu.VMEM((B, 8, W), f32),
                pltpu.VMEM((8, W), bf),
                pltpu.VMEM((8, DH), f32),
                pltpu.VMEM((B, 8, DH), f32),
                pltpu.VMEM((8, D), f32),
                pltpu.VMEM((8, F), bf),
                pltpu.VMEM((8, D), f32),
                pltpu.VMEM((8, F), f32),
                pltpu.SemaphoreType.DMA((R0,)), pltpu.SemaphoreType.DMA((R1,)),
                pltpu.SemaphoreType.DMA((1,)),
            ],
            compiler_params=pltpu.CompilerParams(vmem_limit_bytes=110 * 1024 * 1024,
                                                 disable_bounds_checks=not checks,
                                                 disable_semaphore_checks=not checks),
        )(A_x.reshape(B, D), A_k_cache, A_v_cache, A_wq, A_wo.T, B_w1, B_b1.reshape(F // 128, 128), B_w2.T, B_b2)
        return out.reshape(B, 1, D)

    return fn


_impl = make()


@jax.jit
def pallas_recurrent_scan__sliding_block_cached__dense_activation_gelu__decode_kernel(
    A_x: jax.Array,
    A_k_cache: jax.Array,
    A_v_cache: jax.Array,
    A_wq: jax.Array,
    A_wo: jax.Array,
    B_x: jax.Array,
    B_w1: jax.Array,
    B_b1: jax.Array,
    B_w2: jax.Array,
    B_b2: jax.Array,
):
    return _impl(A_x, A_k_cache, A_v_cache, A_wq, A_wo, B_x, B_w1, B_b1, B_w2, B_b2)
```

```python
import functools
import jax
import jax.numpy as jnp
from jax import lax
from jax.experimental import pallas as pl
from jax.experimental.pallas import tpu as pltpu

B, D, HQ, HKV, SK, DH, F = 2, 576, 32, 16, 32768, 128, 4608
W = 4096
NT = (((1,), (1,)), ((), ()))
NN = (((1,), (0,)), ((), ()))
bf = jnp.bfloat16
f32 = jnp.float32

NJ = 4
NS = 8
U1 = 24
U2 = 8 * HKV
U3A = 12
U3B = (8, 10)
T2 = U1
T3 = T2 + U2
T4 = T3 + U3A
T5 = T4 + U3B[1]
FR0, FRN = 384, 128
C0, C1 = 128, 384
HR = 1024


def _mo(x, m):
    return x if isinstance(x, int) else pl.multiple_of(x, m)


def make(no_dma=False, no_compute=False, A0=2, A1=4, checks=True, blocks=(10, 9, 8, 5, 4), scopes=False, dbg=()):
    AH = (A0, A1)
    NB = len(blocks)
    assert sum(blocks) == F // 128 and NB <= 2 * NJ
    boff = [128 * sum(blocks[:i]) for i in range(NB + 1)]

    def scope(name):
        import contextlib
        return jax.named_scope(name) if scopes else contextlib.nullcontext()

    def kernel(x_hbm, k_hbm, v_hbm, wq_hbm, woT_hbm, w1_hbm, b1_hbm, w2T_hbm, b2_hbm, o_hbm,
               kbuf, vbuf, wqb, wob, w1b, w2b, xb, b1b, b2b, ob,
               x8b, qs, sc, pb, lsum, acc, lbuf, sacc, hb, yb, b1f,
               sem0, sem1, semx, fsem):
        sems = (sem0, sem1)

        def slab(src, dst, r0, sem):
            r0 = _mo(r0, 8)
            return pltpu.make_async_copy(src.at[pl.ds(r0, 8), :], dst.at[pl.ds(r0, 8), :], sem)

        def halfslab(src, dst, r0, hf, sem):
            r0 = _mo(r0, 8)
            half = dst.shape[1] // 2
            return pltpu.make_async_copy(src.at[pl.ds(r0, 8), pl.ds(hf * half, half)], dst.at[pl.ds(r0, 8), pl.ds(hf * half, half)], sem)

        def p1_copies(s, u, j, slot, sub):
            sem = sems[s].at[slot]
            if s == 0:
                return [halfslab(wq_hbm, wqb, 16 * u + 8 * (j // 2), j % 2, sem)]
            if sub == 0:
                return [slab(wq_hbm, wqb, 384 + 32 * u + 8 * j, sem)]
            return [slab(w1_hbm, w1b, 32 * (u - 6) + 8 * j, sem)]

        def p2_copies(s, h, k, j, slot):
            sem = sems[s].at[slot]
            q = 4 * k + j
            if s == 0:
                r0 = q * C0
                return [pltpu.make_async_copy(k_hbm.at[0, h, pl.ds(SK - W + r0, C0), :], kbuf.at[h, 0, pl.ds(r0, C0), :], sem)]
            wins = [(k_hbm, kbuf, 1), (v_hbm, vbuf, 0), (v_hbm, vbuf, 1)]
            out = []
            lo, hi = q * C1, (q + 1) * C1
            while lo < hi:
                w = lo // W
                e = min(hi, (w + 1) * W)
                src, dst, b = wins[w]
                r0 = lo - w * W
                out.append(pltpu.make_async_copy(src.at[b, h, pl.ds(SK - W + r0, e - lo), :], dst.at[h, b, pl.ds(r0, e - lo), :], sem))
                lo = e
            return out

        def p3_copies(s, t, j):
            slot = t % NS
            sem = sems[s].at[slot]
            if t < T4:
                u = t - T3
                if s == 0:
                    return [halfslab(woT_hbm, wob, 16 * u + 8 * (j // 2), j % 2, sem)]
                return [slab(woT_hbm, wob, 192 + 32 * u + 8 * j, sem)]
            u = t - T4
            if s == 0:
                if u >= U3B[0]:
                    return []
                r0 = 16 * u + 8 * (j // 2)
                r0 = 512 + r0 if r0 < 64 else r0 - 64
                return [halfslab(w2T_hbm, w2b, r0, j % 2, sem)]
            if u < U3B[1]:
                return [slab(w2T_hbm, w2b, 64 + 32 * u + 8 * j, sem)]
            i = (u - U3B[1]) * NJ + j
            if i >= NB:
                return []
            cs = pl.ds(boff[i], boff[i + 1] - boff[i])
            return [pltpu.make_async_copy(w2T_hbm.at[pl.ds(FR0, FRN), cs], w2b.at[pl.ds(FR0, FRN), cs], fsem.at[i])]

        def do(cs, what, s):
            if no_dma:
                return
            for c in cs:
                if what == "start":
                    c.start(priority=s)
                else:
                    c.wait()

        def static_copies(s, t, j):
            slot = t % NS
            if t < T2:
                return p1_copies(s, t, j, slot, 0 if t < 6 else 1)
            if t < T3:
                n = t - T2
                return p2_copies(s, n // 8, n % 8, j, slot)
            return p3_copies(s, t, j)

        def step_static(t, j):
            do(static_copies(1, t, j), "wait", 1)
            do(static_copies(0, t + A0, j), "start", 0)
            do(static_copies(0, t, j), "wait", 0)
            do(static_copies(1, t + A1, j), "start", 1)

        def step_p1(t, j):
            do(p1_copies(1, t, j, t & (NS - 1), 1), "wait", 1)
            do(p1_copies(0, t + A0, j, (t + A0) & (NS - 1), 0), "start", 0)
            do(p1_copies(0, t, j, t & (NS - 1), 0), "wait", 0)
            do(p1_copies(1, t + A1, j, (t + A1) & (NS - 1), 1), "start", 1)

        def p2_start(s, h, k, j):
            kk = k + AH[s]
            slot = (T2 + kk) % NS
            if kk < 8:
                do(p2_copies(s, h, kk, j, slot), "start", s)
            else:
                pl.when(h < HKV - 1)(lambda: do(p2_copies(s, h + 1, kk - 8, j, slot), "start", s))
                pl.when(h == HKV - 1)(lambda: do(p3_copies(s, T3 + kk - 8, j), "start", s))

        def step_p2(h, k, j):
            slot = (T2 + k) % NS
            do(p2_copies(1, h, k, j, slot), "wait", 1)
            p2_start(0, h, k, j)
            do(p2_copies(0, h, k, j, slot), "wait", 0)
            p2_start(1, h, k, j)

        def unit(stepf, slots=None):
            for j in range(NJ):
                stepf(j)
                if slots is not None and not no_compute:
                    for fn_ in slots.get(j, ()):
                        fn_()

        cx = pltpu.make_async_copy(x_hbm, xb, semx.at[0])
        cb1 = pltpu.make_async_copy(b1_hbm, b1b, semx.at[0])
        cb2 = pltpu.make_async_copy(b2_hbm, b2b, semx.at[0])
        for t in range(A0):
            for j in range(NJ):
                do(static_copies(0, t, j), "start", 0)
        if not no_dma:
            cx.start(); cb1.start(); cb2.start()
        for t in range(A1):
            for j in range(NJ):
                do(static_copies(1, t, j), "start", 1)

        row128 = lax.broadcasted_iota(jnp.int32, (8, DH), 0)

        def prep():
            if not no_dma:
                cx.wait(); cb1.wait(); cb2.wait()
            x = xb[...].astype(f32)
            mu = jnp.mean(x, axis=-1, keepdims=True)
            xc = x - mu
            var = jnp.mean(xc * xc, axis=-1, keepdims=True)
            xn = xc / jnp.sqrt(var + 1e-5)
            rowd = lax.broadcasted_iota(jnp.int32, (8, D), 0)
            x8b[...] = jnp.where(rowd % 2 == 0, jnp.broadcast_to(xn[0:1], (8, D)), jnp.broadcast_to(xn[1:2], (8, D))).astype(bf)
            bias1 = b1b[...].astype(f32)
            for j in range(F // 128):
                b1f[:, pl.ds(128 * j, 128)] = jnp.broadcast_to(bias1[j:j + 1, :], (8, 128))

        def qproj(h):
            c0 = _mo(h * 256, 256)
            q = lax.dot_general(x8b[...], wqb[:, pl.ds(c0, 256)], NN, preferred_element_type=f32)
            qs[h] = jnp.where(row128 < 2, q[:, :128], q[:, 128:]).astype(bf)

        def ffn1(p):
            c0 = _mo(p * 256, 256)
            hh = lax.dot_general(x8b[...], w1b[:, pl.ds(c0, 256)], NN, preferred_element_type=f32)
            hh = hh + b1f[:, pl.ds(c0, 256)]
            hb[:, pl.ds(c0, 256)] = jax.nn.gelu(hh, approximate=True).astype(bf)

        def qk(h, b, q4):
            s = lax.dot_general(qs[h], kbuf[h, b, pl.ds(q4 * HR, HR), :], NT, preferred_element_type=f32)
            sc[b, :, pl.ds(q4 * HR, HR)] = s

        def softmax():
            roww = lax.broadcasted_iota(jnp.int32, (8, W), 0)
            s = jnp.where(roww % 2 == 0, sc[0], sc[1]) * (DH ** -0.5)
            m = jnp.max(s, axis=-1, keepdims=True)
            p = jnp.exp(s - m)
            l = jnp.sum(p, axis=-1, keepdims=True)
            lsum[...] = jnp.broadcast_to(l, (8, DH))
            pb[...] = p.astype(bf)

        def pv(h, b, q4):
            o = lax.dot_general(pb[:, pl.ds(q4 * HR, HR)], vbuf[h, b, pl.ds(q4 * HR, HR), :], NN, preferred_element_type=f32)
            if q4 == 0:
                acc[b] = o
            else:
                acc[b] = acc[b] + o

        def finalize(h):
            o = jnp.where(row128 % 2 == 0, acc[0], acc[1]) / lsum[...]
            la = jnp.where(row128 < 2, o, 0.0)
            lb = jnp.where((row128 >= 2) & (row128 < 4), o, 0.0)
            c0 = _mo(h * 256, 256)
            lbuf[:, pl.ds(c0, 256)] = jnp.concatenate([la, lb], axis=1).astype(bf)

        def wopiece(p):
            sacc[:, pl.ds(64 * p, 64)] = lax.dot_general(lbuf[...], wob[pl.ds(64 * p, 64), :], NT, preferred_element_type=f32)

        def ffn2(p):
            yb[:, pl.ds(64 * p, 64)] = lax.dot_general(hb[...], w2b[pl.ds(64 * p, 64), :], NT, preferred_element_type=f32)

        def silu(y):
            return y * (0.5 * jnp.tanh(0.5 * y) + 0.5)

        def attn_slot(h, sg):
            out = []
            if sg % 2 == 0:
                i = sg // 2
                if i < 8:
                    out.append(functools.partial(qk, h, i // 4, i % 4))
                else:
                    out.append(functools.partial(pv, h, (i - 8) // 4, i % 4))
            if sg == 15:
                out.append(softmax)
            if sg == 31:
                out.append(functools.partial(finalize, h))
            return out

        NPEEL = max(A0, A1)
        with scope("ph1"):
            unit(lambda j: step_static(0, j))
            if not no_compute:
                prep()
            elif not no_dma:
                cx.wait(); cb1.wait(); cb2.wait()
            for t in range(1, 6):
                unit(lambda j, t=t: step_static(t, j))

            def body1(t, c):
                unit(lambda j: step_p1(t, j))
                return c
            lax.fori_loop(6, T2 - NPEEL, body1, 0)
            for t in range(T2 - NPEEL, T2):
                unit(lambda j, t=t: step_static(t, j))

        def body2(h, c):
            for k in range(8):
                slots = {}
                for j in range(NJ):
                    sg = 4 * k + j
                    fns = attn_slot(h - 1, sg)
                    lst = []
                    if fns:
                        lst.append(lambda fns=fns: pl.when(h > 0)(lambda: [f() for f in fns] and None))
                    if sg == 5:
                        lst.append(lambda: pl.when(h >= 0)(lambda: qproj(h)))
                    if sg % 2 == 1 and sg not in (5, 15, 31) and sg >= 7:
                        ii = [x for x in range(7, 31, 2) if x != 15].index(sg)
                        if ii < 9:
                            lst.append(lambda ii=ii: pl.when(h < 2)(lambda: ffn1(9 * h + ii)))
                    if lst:
                        slots[j] = lst
                with scope("p2"):
                    unit(lambda j, k=k: step_p2(h, k, j), slots)
            return c
        lax.fori_loop(0, HKV, body2, 0)

        h = HKV - 1
        wo_ready = {0: 3, 1: 7, 2: 11, 3: 1, 4: 3, 5: 5, 6: 7, 7: 9, 8: 11}
        f2_ready = {8: 3, 0: 7, 1: 1, 2: 3, 3: 5, 4: 7, 5: 9}
        heavy = [(max(T3 + r, T3 + 7), functools.partial(wopiece, p)) for p, r in wo_ready.items()]
        heavy += [(T4 + r, functools.partial(ffn2, p)) for p, r in f2_ready.items()]
        heavy.sort(key=lambda x: x[0])
        for t in range(T3, T5):
            u = t - T3
            slots = {}
            nh = 0
            for j in range(NJ):
                fns = list(attn_slot(h, 4 * u + j)) if u < 8 else []
                if not fns and nh < 2 and (j % 2 == 1):
                    avail = [x for x in heavy if x[0] < t]
                    if avail:
                        heavy.remove(avail[0])
                        fns.append(avail[0][1])
                        nh += 1
                if fns:
                    slots[j] = fns
            with scope("p3u%d" % u):
                unit(lambda j, t=t: step_static(t, j), slots)

        x = xb[...].astype(f32)
        b2 = b2b[...].astype(f32).reshape(1, D)
        if not no_compute:
            with scope("lastheavy"):
                for _, fn_ in heavy:
                    fn_()
            with scope("fin"):
                s8 = sacc[...]
                sres = s8[0:2] + s8[2:4]
                for lo, hi in ((0, FR0), (FR0 + FRN, D)):
                    y0 = yb[0:2, lo:hi] + b2[:, lo:hi]
                    ob[:, lo:hi] = (x[:, lo:hi] + sres[:, lo:hi] * silu(y0)).astype(bf)
                yl = jnp.broadcast_to(b2[:, FR0:FR0 + FRN], (8, FRN))
        for i in range(NB):
            with scope("bw%d" % i):
                do(static_copies(1, T5 + i // NJ, i % NJ), "wait", 1)
            if not no_compute:
                with scope("bc%d" % i):
                    cs = pl.ds(boff[i], boff[i + 1] - boff[i])
                    yl = yl + lax.dot_general(hb[:, cs], w2b[pl.ds(FR0, FRN), cs], NT, preferred_element_type=f32)
        if not no_compute:
            ob[:, FR0:FR0 + FRN] = (x[:, FR0:FR0 + FRN] + sres[:, FR0:FR0 + FRN] * silu(yl[0:2])).astype(bf)
        else:
            ob[...] = x.astype(bf)
        with scope("outdma"):
            oc = pltpu.make_async_copy(ob, o_hbm, semx.at[0])
            oc.start(); oc.wait()

    @jax.jit
    def fn(A_x, A_k_cache, A_v_cache, A_wq, A_wo, B_x, B_w1, B_b1, B_w2, B_b2):
        hbm = pl.BlockSpec(memory_space=pltpu.HBM)
        out = pl.pallas_call(
            kernel,
            out_shape=jax.ShapeDtypeStruct((B, D), bf),
            in_specs=[hbm] * 9,
            out_specs=hbm,
            scratch_shapes=[
                pltpu.VMEM((HKV, B, W, DH), bf), pltpu.VMEM((HKV, B, W, DH), bf),
                pltpu.VMEM((D, HQ * DH), bf), pltpu.VMEM((D, HQ * DH), bf),
                pltpu.VMEM((D, F), bf), pltpu.VMEM((D, F), bf),
                pltpu.VMEM((B, D), bf), pltpu.VMEM((F // 128, 128), bf), pltpu.VMEM((D,), bf),
                pltpu.VMEM((B, D), bf),
                pltpu.VMEM((8, D), bf),
                pltpu.VMEM((HKV, 8, DH), bf),
                pltpu.VMEM((B, 8, W), f32),
                pltpu.VMEM((8, W), bf),
                pltpu.VMEM((8, DH), f32),
                pltpu.VMEM((B, 8, DH), f32),
                pltpu.VMEM((8, HQ * DH), bf),
                pltpu.VMEM((8, D), f32),
                pltpu.VMEM((8, F), bf),
                pltpu.VMEM((8, D), f32),
                pltpu.VMEM((8, F), f32),
                pltpu.SemaphoreType.DMA((NS,)), pltpu.SemaphoreType.DMA((NS,)),
                pltpu.SemaphoreType.DMA((1,)), pltpu.SemaphoreType.DMA((2 * NJ,)),
            ],
            compiler_params=pltpu.CompilerParams(vmem_limit_bytes=110 * 1024 * 1024,
                                                 disable_bounds_checks=not checks,
                                                 disable_semaphore_checks=not checks),
        )(A_x.reshape(B, D), A_k_cache, A_v_cache, A_wq, A_wo.T, B_w1, B_b1.reshape(F // 128, 128), B_w2.T, B_b2)
        return out.reshape(B, 1, D)

    return fn


_impl = make(checks=False)


@jax.jit
def pallas_recurrent_scan__sliding_block_cached__dense_activation_gelu__decode_kernel(
    A_x: jax.Array,
    A_k_cache: jax.Array,
    A_v_cache: jax.Array,
    A_wq: jax.Array,
    A_wo: jax.Array,
    B_x: jax.Array,
    B_w1: jax.Array,
    B_b1: jax.Array,
    B_w2: jax.Array,
    B_b2: jax.Array,
):
    return _impl(A_x, A_k_cache, A_v_cache, A_wq, A_wo, B_x, B_w1, B_b1, B_w2, B_b2)
```

```python
import functools

import jax
import jax.numpy as jnp
from jax import lax
from jax.experimental import pallas as pl
from jax.experimental.pallas import tpu as pltpu

B, D, HQ, HKV, SK, DH, F = 2, 576, 32, 16, 32768, 128, 4608
W = 4096
NT = (((1,), (1,)), ((), ()))
NN = (((1,), (0,)), ((), ()))
bf = jnp.bfloat16
f32 = jnp.float32

NJ = 4
NS = 8
A0, A1 = 2, 4
U1 = 24
U2 = 8 * HKV
U3A = 12
U3B = (8, 10)
T2 = U1
T3 = T2 + U2
T4 = T3 + U3A
T5 = T4 + U3B[1]
FR0, FRN = 384, 128
BLOCKS = (10, 9, 8, 5, 4)
NB = len(BLOCKS)
BOFF = [128 * sum(BLOCKS[:i]) for i in range(NB + 1)]
C0, C1 = 128, 384
HR = 1024


def _mo(x, m):
    return x if isinstance(x, int) else pl.multiple_of(x, m)


def _kernel(x_hbm, k_hbm, v_hbm, wq_hbm, woT_hbm, w1_hbm, b1_hbm, w2T_hbm, b2_hbm, o_hbm,
            kbuf, vbuf, wqb, wob, w1b, w2b, xb, b1b, b2b, ob,
            x8b, qs, sc, pb, lsum, acc, lbuf, sacc, hb, yb, b1f,
            sem0, sem1, semx, fsem):
    sems = (sem0, sem1)
    look = (A0, A1)

    def slab(src, dst, r0, sem):
        rows = pl.ds(_mo(r0, 8), 8)
        return pltpu.make_async_copy(src.at[rows, :], dst.at[rows, :], sem)

    def halfslab(src, dst, r0, hf, sem):
        rows = pl.ds(_mo(r0, 8), 8)
        half = dst.shape[1] // 2
        cols = pl.ds(hf * half, half)
        return pltpu.make_async_copy(src.at[rows, cols], dst.at[rows, cols], sem)

    def p1_copies(s, u, j, slot, on_w1):
        sem = sems[s].at[slot]
        if s == 0:
            return [halfslab(wq_hbm, wqb, 16 * u + 8 * (j // 2), j % 2, sem)]
        if not on_w1:
            return [slab(wq_hbm, wqb, 384 + 32 * u + 8 * j, sem)]
        return [slab(w1_hbm, w1b, 32 * (u - 6) + 8 * j, sem)]

    def p2_copies(s, h, k, j, slot):
        sem = sems[s].at[slot]
        q = NJ * k + j
        if s == 0:
            pieces = [(k_hbm, kbuf, 0, q * C0, C0)]
        else:
            wins = [(k_hbm, kbuf, 1), (v_hbm, vbuf, 0), (v_hbm, vbuf, 1)]
            pieces = []
            lo, hi = q * C1, (q + 1) * C1
            while lo < hi:
                w = lo // W
                e = min(hi, (w + 1) * W)
                pieces.append(wins[w] + (lo - w * W, e - lo))
                lo = e
        return [pltpu.make_async_copy(src.at[b, h, pl.ds(SK - W + r0, n), :], dst.at[h, b, pl.ds(r0, n), :], sem)
                for src, dst, b, r0, n in pieces]

    def p3_copies(s, t, j):
        sem = sems[s].at[t % NS]
        if t < T4:
            u = t - T3
            if s == 0:
                return [halfslab(woT_hbm, wob, 16 * u + 8 * (j // 2), j % 2, sem)]
            return [slab(woT_hbm, wob, 192 + 32 * u + 8 * j, sem)]
        u = t - T4
        if s == 0:
            if u >= U3B[0]:
                return []
            r0 = 16 * u + 8 * (j // 2)
            return [halfslab(w2T_hbm, w2b, 512 + r0 if r0 < 64 else r0 - 64, j % 2, sem)]
        if u < U3B[1]:
            return [slab(w2T_hbm, w2b, 64 + 32 * u + 8 * j, sem)]
        i = (u - U3B[1]) * NJ + j
        if i >= NB:
            return []
        rows, cols = pl.ds(FR0, FRN), pl.ds(BOFF[i], BOFF[i + 1] - BOFF[i])
        return [pltpu.make_async_copy(w2T_hbm.at[rows, cols], w2b.at[rows, cols], fsem.at[i])]

    def static_copies(s, t, j):
        if t < T2:
            return p1_copies(s, t, j, t % NS, t >= 6)
        if t < T3:
            n = t - T2
            return p2_copies(s, n // 8, n % 8, j, t % NS)
        return p3_copies(s, t, j)

    def start(copies, s):
        for c in copies:
            c.start(priority=s)

    def wait(copies):
        for c in copies:
            c.wait()

    def step_static(t, j):
        wait(static_copies(1, t, j))
        start(static_copies(0, t + A0, j), 0)
        wait(static_copies(0, t, j))
        start(static_copies(1, t + A1, j), 1)

    def step_p1(t, j):
        wait(p1_copies(1, t, j, t & (NS - 1), True))
        start(p1_copies(0, t + A0, j, (t + A0) & (NS - 1), True), 0)
        wait(p1_copies(0, t, j, t & (NS - 1), True))
        start(p1_copies(1, t + A1, j, (t + A1) & (NS - 1), True), 1)

    def p2_start(s, h, k, j):
        kk = k + look[s]
        slot = (T2 + kk) % NS
        if kk < 8:
            start(p2_copies(s, h, kk, j, slot), s)
        else:
            pl.when(h < HKV - 1)(lambda: start(p2_copies(s, h + 1, kk - 8, j, slot), s))
            pl.when(h == HKV - 1)(lambda: start(p3_copies(s, T3 + kk - 8, j), s))

    def step_p2(h, k, j):
        slot = (T2 + k) % NS
        wait(p2_copies(1, h, k, j, slot))
        p2_start(0, h, k, j)
        wait(p2_copies(0, h, k, j, slot))
        p2_start(1, h, k, j)

    def unit(stepf, slots=None):
        for j in range(NJ):
            stepf(j)
            for fn in (slots or {}).get(j, ()):
                fn()

    small = [pltpu.make_async_copy(x_hbm, xb, semx.at[0]),
             pltpu.make_async_copy(b1_hbm, b1b, semx.at[0]),
             pltpu.make_async_copy(b2_hbm, b2b, semx.at[0])]
    for t in range(A0):
        for j in range(NJ):
            start(static_copies(0, t, j), 0)
    start(small, 0)
    for t in range(A1):
        for j in range(NJ):
            start(static_copies(1, t, j), 1)

    row128 = lax.broadcasted_iota(jnp.int32, (8, DH), 0)

    def prep():
        wait(small)
        x = xb[...].astype(f32)
        mu = jnp.mean(x, axis=-1, keepdims=True)
        xc = x - mu
        var = jnp.mean(xc * xc, axis=-1, keepdims=True)
        xn = xc / jnp.sqrt(var + 1e-5)
        rowd = lax.broadcasted_iota(jnp.int32, (8, D), 0)
        x8b[...] = jnp.where(rowd % 2 == 0, jnp.broadcast_to(xn[0:1], (8, D)),
                             jnp.broadcast_to(xn[1:2], (8, D))).astype(bf)
        bias1 = b1b[...].astype(f32)
        for j in range(F // 128):
            b1f[:, pl.ds(128 * j, 128)] = jnp.broadcast_to(bias1[j:j + 1, :], (8, 128))

    def qproj(h):
        cols = pl.ds(_mo(h * 256, 256), 256)
        q = lax.dot_general(x8b[...], wqb[:, cols], NN, preferred_element_type=f32)
        qs[h] = jnp.where(row128 < 2, q[:, :128], q[:, 128:]).astype(bf)

    def ffn1(p):
        cols = pl.ds(_mo(p * 256, 256), 256)
        hh = lax.dot_general(x8b[...], w1b[:, cols], NN, preferred_element_type=f32) + b1f[:, cols]
        hb[:, cols] = jax.nn.gelu(hh, approximate=True).astype(bf)

    def qk(h, b, i):
        rows = pl.ds(i * HR, HR)
        sc[b, :, rows] = lax.dot_general(qs[h], kbuf[h, b, rows, :], NT, preferred_element_type=f32)

    def softmax():
        roww = lax.broadcasted_iota(jnp.int32, (8, W), 0)
        s = jnp.where(roww % 2 == 0, sc[0], sc[1]) * (DH ** -0.5)
        m = jnp.max(s, axis=-1, keepdims=True)
        p = jnp.exp(s - m)
        lsum[...] = jnp.broadcast_to(jnp.sum(p, axis=-1, keepdims=True), (8, DH))
        pb[...] = p.astype(bf)

    def pv(h, b, i):
        rows = pl.ds(i * HR, HR)
        o = lax.dot_general(pb[:, rows], vbuf[h, b, rows, :], NN, preferred_element_type=f32)
        acc[b] = o if i == 0 else acc[b] + o

    def finalize(h):
        o = jnp.where(row128 % 2 == 0, acc[0], acc[1]) / lsum[...]
        la = jnp.where(row128 < 2, o, 0.0)
        lb = jnp.where((row128 >= 2) & (row128 < 4), o, 0.0)
        lbuf[:, pl.ds(_mo(h * 256, 256), 256)] = jnp.concatenate([la, lb], axis=1).astype(bf)

    def wo_piece(p):
        sacc[:, pl.ds(64 * p, 64)] = lax.dot_general(lbuf[...], wob[pl.ds(64 * p, 64), :], NT,
                                                     preferred_element_type=f32)

    def ffn2(p):
        yb[:, pl.ds(64 * p, 64)] = lax.dot_general(hb[...], w2b[pl.ds(64 * p, 64), :], NT,
                                                   preferred_element_type=f32)

    def silu(y):
        return y * (0.5 * jnp.tanh(0.5 * y) + 0.5)

    def attn_slot(h, sg):
        np_ = W // HR
        out = []
        if sg % 2 == 0:
            i = sg // 2
            if i < 2 * np_:
                out.append(functools.partial(qk, h, i // np_, i % np_))
            else:
                out.append(functools.partial(pv, h, (i - 2 * np_) // np_, i % np_))
        if sg == 15:
            out.append(softmax)
        if sg == 31:
            out.append(functools.partial(finalize, h))
        return out

    def run_all(fns):
        for fn in fns:
            fn()

    npeel = max(A0, A1)
    unit(lambda j: step_static(0, j))
    prep()
    for t in range(1, 6):
        unit(functools.partial(step_static, t))

    def body1(t, c):
        unit(functools.partial(step_p1, t))
        return c

    lax.fori_loop(6, T2 - npeel, body1, 0)
    for t in range(T2 - npeel, T2):
        unit(functools.partial(step_static, t))

    ffn1_slots = [x for x in range(7, 31, 2) if x != 15][:9]

    def body2(h, c):
        for k in range(8):
            slots = {}
            for j in range(NJ):
                sg = NJ * k + j
                lst = []
                fns = attn_slot(h - 1, sg)
                if fns:
                    lst.append(lambda fns=fns: pl.when(h > 0)(lambda: run_all(fns)))
                if sg == 5:
                    lst.append(lambda: pl.when(h >= 0)(lambda: qproj(h)))
                if sg in ffn1_slots:
                    ii = ffn1_slots.index(sg)
                    lst.append(lambda ii=ii: pl.when(h < 2)(lambda: ffn1(9 * h + ii)))
                if lst:
                    slots[j] = lst
            unit(functools.partial(step_p2, h, k), slots)
        return c

    lax.fori_loop(0, HKV, body2, 0)

    wo_ready = {0: 3, 1: 7, 2: 11, 3: 1, 4: 3, 5: 5, 6: 7, 7: 9, 8: 11}
    f2_ready = {8: 3, 0: 7, 1: 1, 2: 3, 3: 5, 4: 7, 5: 9}
    heavy = [(max(T3 + r, T3 + 7), functools.partial(wo_piece, p)) for p, r in wo_ready.items()]
    heavy += [(T4 + r, functools.partial(ffn2, p)) for p, r in f2_ready.items()]
    heavy.sort(key=lambda e: e[0])
    for t in range(T3, T5):
        u = t - T3
        slots = {}
        for j in range(NJ):
            fns = attn_slot(HKV - 1, NJ * u + j) if u < 8 else []
            if not fns and j % 2 == 1:
                avail = [e for e in heavy if e[0] < t]
                if avail:
                    heavy.remove(avail[0])
                    fns = [avail[0][1]]
            if fns:
                slots[j] = fns
        unit(functools.partial(step_static, t), slots)

    x = xb[...].astype(f32)
    b2 = b2b[...].astype(f32).reshape(1, D)
    run_all([e[1] for e in heavy])
    s8 = sacc[...]
    sres = s8[0:2] + s8[2:4]
    for lo, hi in ((0, FR0), (FR0 + FRN, D)):
        ob[:, lo:hi] = (x[:, lo:hi] + sres[:, lo:hi] * silu(yb[0:2, lo:hi] + b2[:, lo:hi])).astype(bf)
    yl = jnp.broadcast_to(b2[:, FR0:FR0 + FRN], (8, FRN))
    for i in range(NB):
        wait(static_copies(1, T5 + i // NJ, i % NJ))
        cols = pl.ds(BOFF[i], BOFF[i + 1] - BOFF[i])
        yl = yl + lax.dot_general(hb[:, cols], w2b[pl.ds(FR0, FRN), cols], NT, preferred_element_type=f32)
    ob[:, FR0:FR0 + FRN] = (x[:, FR0:FR0 + FRN] + sres[:, FR0:FR0 + FRN] * silu(yl[0:2])).astype(bf)
    out_copy = pltpu.make_async_copy(ob, o_hbm, semx.at[0])
    out_copy.start()
    out_copy.wait()


@jax.jit
def pallas_recurrent_scan__sliding_block_cached__dense_activation_gelu__decode_kernel(
    A_x: jax.Array,
    A_k_cache: jax.Array,
    A_v_cache: jax.Array,
    A_wq: jax.Array,
    A_wo: jax.Array,
    B_x: jax.Array,
    B_w1: jax.Array,
    B_b1: jax.Array,
    B_w2: jax.Array,
    B_b2: jax.Array,
):
    del B_x
    hbm = pl.BlockSpec(memory_space=pltpu.HBM)
    out = pl.pallas_call(
        _kernel,
        out_shape=jax.ShapeDtypeStruct((B, D), bf),
        in_specs=[hbm] * 9,
        out_specs=hbm,
        scratch_shapes=[
            pltpu.VMEM((HKV, B, W, DH), bf),
            pltpu.VMEM((HKV, B, W, DH), bf),
            pltpu.VMEM((D, HQ * DH), bf),
            pltpu.VMEM((D, HQ * DH), bf),
            pltpu.VMEM((D, F), bf),
            pltpu.VMEM((D, F), bf),
            pltpu.VMEM((B, D), bf),
            pltpu.VMEM((F // 128, 128), bf),
            pltpu.VMEM((D,), bf),
            pltpu.VMEM((B, D), bf),
            pltpu.VMEM((8, D), bf),
            pltpu.VMEM((HKV, 8, DH), bf),
            pltpu.VMEM((B, 8, W), f32),
            pltpu.VMEM((8, W), bf),
            pltpu.VMEM((8, DH), f32),
            pltpu.VMEM((B, 8, DH), f32),
            pltpu.VMEM((8, HQ * DH), bf),
            pltpu.VMEM((8, D), f32),
            pltpu.VMEM((8, F), bf),
            pltpu.VMEM((8, D), f32),
            pltpu.VMEM((8, F), f32),
            pltpu.SemaphoreType.DMA((NS,)),
            pltpu.SemaphoreType.DMA((NS,)),
            pltpu.SemaphoreType.DMA((1,)),
            pltpu.SemaphoreType.DMA((NB,)),
        ],
        compiler_params=pltpu.CompilerParams(
            vmem_limit_bytes=110 * 1024 * 1024,
            disable_bounds_checks=True,
            disable_semaphore_checks=True,
        ),
    )(A_x.reshape(B, D), A_k_cache, A_v_cache, A_wq, A_wo.T, B_w1, B_b1.reshape(F // 128, 128), B_w2.T, B_b2)
    return out.reshape(B, 1, D)
```
